```python
import jax
import jax.numpy as jnp

def _softmax(x, axis=-1):
    return jax.nn.softmax(x, axis=axis)

def _gelu(x):
    return jax.nn.gelu(x, approximate=True)

def _silu(x):
    return jax.nn.silu(x)

def _sigmoid(x):
    return jax.nn.sigmoid(x)

def _layernorm(x, axis=-1, eps=1e-05):
    m = jnp.mean(x, axis=axis, keepdims=True)
    v = jnp.var(x, axis=axis, keepdims=True)
    return (x - m) / jnp.sqrt(v + eps)

def _scatter_add(tgt, idx, src, axis=0):
    return tgt.at[idx].add(src)

def _segment_sum(src, seg, n):
    return jax.ops.segment_sum(src, seg, n)

class _Rng:

    def __init__(self, key):
        self._k = key

    def _next(self):
        self._k, sub = jax.random.split(self._k)
        return sub

    def normal(self, shape):
        return jax.random.normal(self._next(), shape, dtype=jnp.bfloat16)

    def randint(self, lo, hi, shape):
        return jax.random.randint(self._next(), shape, lo, hi, dtype=jnp.int32)

    def uniform(self, shape, lo=0.0, hi=1.0):
        return jax.random.uniform(self._next(), shape, jnp.bfloat16, lo, hi)

    def permutation(self, n):
        return jax.random.permutation(self._next(), n)
kernel_name = 'interleave_layers__linear_kernel_hedgehog__mixer_gmlp__prompt'

def _fwd_setup_inputs():
    _rng = _Rng(jax.random.key(int.from_bytes(__import__("os").urandom(4), "little")))
    _w = lambda a: (lambda t: t.astype(jnp.bfloat16) if jnp.issubdtype(t.dtype, jnp.floating) else t)(jnp.asarray(a))

    def _A_setup():
        B, S, D, H = (1, 2048, 640, 32)
        Dh = D // H
        return {'x': _w((lambda *s: _rng.normal(s) * 0.05)(B, S, D)), 'wqkv': _w((lambda *s: _rng.normal(s) * 0.05)(D, 3 * D)), 'w_phi': _w((lambda *s: _rng.normal(s) * 0.05)(H, Dh, Dh) * Dh ** (-0.5)), 'wo': _w((lambda *s: _rng.normal(s) * 0.05)(D, D))}
    _A_in = _A_setup()

    def _B_setup():
        B, S, D, F = (1, 2048, 640, 1536)
        Fh = F // 2
        return {'x': _w((lambda *s: _rng.normal(s) * 0.05)(B, S, D)), 'w_in': _w((lambda *s: _rng.normal(s) * 0.05)(D, 2 * Fh)), 'w_sp': _w(0.01 * (lambda *s: _rng.normal(s) * 0.05)(S, S)), 'b_sp': _w(1.0 + 0.01 * (lambda *s: _rng.normal(s) * 0.05)(S)), 'w_out': _w((lambda *s: _rng.normal(s) * 0.05)(Fh, D))}
    _B_in = _B_setup()
    return {'A_x': _A_in['x'], 'A_wqkv': _A_in['wqkv'], 'A_w_phi': _A_in['w_phi'], 'A_wo': _A_in['wo'], 'B_x': _B_in['x'], 'B_w_in': _B_in['w_in'], 'B_w_sp': _B_in['w_sp'], 'B_b_sp': _B_in['b_sp'], 'B_w_out': _B_in['w_out']}

def _fwd_reference(A_x, A_wqkv, A_w_phi, A_wo, B_x, B_w_in, B_w_sp, B_b_sp, B_w_out):

    def _A_ref(x, wqkv, w_phi, wo):
        B, S, D = x.shape
        H = 32
        Dh = D // H
        qkv = (lambda x, *d: x.transpose(*d))((x @ wqkv).reshape(B, S, 3, H, Dh), 2, 0, 3, 1, 4)
        q, k, v = (qkv[0], qkv[1], qkv[2])
        pq = jnp.einsum('bhsd,hdf->bhsf', q, w_phi)
        pk = jnp.einsum('bhsd,hdf->bhsf', k, w_phi)
        phi_q = jnp.concatenate([_softmax(pq, axis=-1), _softmax(-pq, axis=-1)], axis=-1)
        phi_k = jnp.concatenate([_softmax(pk, axis=-1), _softmax(-pk, axis=-1)], axis=-1)
        kv = jnp.einsum('bhsf,bhsd->bhfd', phi_k, v)
        z = jnp.einsum('bhsf->bhf', phi_k)
        num = jnp.einsum('bhqf,bhfd->bhqd', phi_q, kv)
        den = jnp.einsum('bhqf,bhf->bhq', phi_q, z)[..., None] + 1e-06
        o = num / den
        return (lambda x, *d: x.transpose(*d))(o, 0, 2, 1, 3).reshape(B, S, D) @ wo

    def _B_ref(x, w_in, w_sp, b_sp, w_out):
        B, S, D = x.shape
        F = w_in.shape[-1]
        Fh = F // 2
        z = _gelu(jnp.einsum('bsd,df->bsf', x, w_in))
        z1 = z[..., :Fh].copy()
        z2 = _layernorm(z[..., Fh:], axis=-1)
        g = jnp.einsum('ts,bsf->btf', w_sp, z2) + b_sp[None, :, None]
        return jnp.einsum('bsf,fd->bsd', z1 * g, w_out)
    x = A_x
    x = x + _A_ref(_layernorm(x, axis=-1), A_wqkv, A_w_phi, A_wo)
    x = x + _B_ref(_layernorm(x, axis=-1), B_w_in, B_w_sp, B_b_sp, B_w_out)
    x = x + _A_ref(_layernorm(x, axis=-1), A_wqkv, A_w_phi, A_wo)
    x = x + _B_ref(_layernorm(x, axis=-1), B_w_in, B_w_sp, B_b_sp, B_w_out)
    return x

def setup_inputs():
    _inp = _fwd_setup_inputs()
    _gk = jax.random.fold_in(jax.random.key(int.from_bytes(__import__("os").urandom(4), "little")), 2 ** 31 - 1)
    _shapes = [[1, 2048, 640]]
    _dtypes = ['bfloat16']
    _gks = jax.random.split(_gk, len(_shapes))
    _gs = [jax.random.normal(k, s, dtype=jnp.dtype(d)) * 0.05 for k, s, d in zip(_gks, _shapes, _dtypes)]
    _inp['grad_out'] = _gs[0]
    return _inp

def reference(A_x, A_wqkv, A_w_phi, A_wo, B_w_in, B_w_sp, B_b_sp, B_w_out, B_x, grad_out):
    _const = dict(B_x=B_x)

    def _f(*_d):
        return _fwd_reference(**{'A_x': _d[0], 'A_wqkv': _d[1], 'A_w_phi': _d[2], 'A_wo': _d[3], 'B_w_in': _d[4], 'B_w_sp': _d[5], 'B_b_sp': _d[6], 'B_w_out': _d[7], **_const})
    _out, _vjp = jax.vjp(_f, A_x, A_wqkv, A_w_phi, A_wo, B_w_in, B_w_sp, B_b_sp, B_w_out)
    _grads = _vjp(grad_out)
    _out0 = jnp.asarray(_out)
    return (_out0, *[jnp.asarray(_g) for _g in _grads])
```

```python
import jax
import jax.numpy as jnp
from jax import lax
import jax.experimental.pallas as pl
import jax.experimental.pallas.tpu as pltpu

f32 = jnp.float32
bf16 = jnp.bfloat16

S = 2048
D = 640
H = 32
DH = 20
FH = 768
NG = 4
GR = 160
GA = 176
C = 512
NC = S // C

A_XN, A_PQ, A_PK, A_O, A_V = 0, 640, 1280, 1920, 2560
A_ROWS = A_V + NG * GA
B_XN, B_H, B_Z2, B_G = 0, 640, 640 + 1536, 640 + 1536 + 768
B_ROWS = B_G + FH

_GC = 0.7978845608028654
_GA3 = 0.044715


def _nn(a, b):
    return jnp.dot(a, b, preferred_element_type=f32)


def _nt(a, b):
    return lax.dot_general(a, b, (((1,), (1,)), ((), ())), preferred_element_type=f32)


def _ln_fwd(x):
    mu = jnp.mean(x, axis=0, keepdims=True)
    xc = x - mu
    var = jnp.mean(xc * xc, axis=0, keepdims=True)
    rstd = lax.rsqrt(var + 1e-5)
    return xc * rstd, rstd


def _ln_bwd(dxn, xn, rstd):
    m1 = jnp.mean(dxn, axis=0, keepdims=True)
    m2 = jnp.mean(dxn * xn, axis=0, keepdims=True)
    return rstd * (dxn - m1 - xn * m2)


def _gelu(x):
    t = jnp.tanh(_GC * (x + _GA3 * (x * x * x)))
    return 0.5 * x * (1.0 + t)


def _gelu_and_grad(x):
    x2 = x * x
    t = jnp.tanh(_GC * (x + _GA3 * (x2 * x)))
    hp = 0.5 * (1.0 + t)
    y = x * hp
    dy = hp + 0.5 * x * (1.0 - t * t) * (_GC * (1.0 + 3.0 * _GA3 * x2))
    return y, dy


def _phi_pair(p):
    n = p.shape[-1]
    p3 = p.reshape(DH, 8, n)
    mx = jnp.max(p3, axis=0, keepdims=True)
    mn = jnp.min(p3, axis=0, keepdims=True)
    ep = jnp.exp(p3 - mx)
    en = jnp.exp(mn - p3)
    sp = jnp.sum(ep, axis=0, keepdims=True)
    sn = jnp.sum(en, axis=0, keepdims=True)
    return ep * (1.0 / sp), en * (1.0 / sn)


def _phi_cat(php, phn):
    n = php.shape[-1]
    return jnp.concatenate(
        [php.reshape(GR, n).astype(bf16), phn.reshape(GR, n).astype(bf16)], axis=0)


def _softmax_pair_bwd(php, phn, dphi):
    n = dphi.shape[-1]
    dp_ = dphi[:GR].reshape(DH, 8, n)
    dn_ = dphi[GR:].reshape(DH, 8, n)
    sp = jnp.sum(php * dp_, axis=0, keepdims=True)
    sn = jnp.sum(phn * dn_, axis=0, keepdims=True)
    return (php * (dp_ - sp) - phn * (dn_ - sn)).reshape(GR, n)


def _kernel(x_ref, wqkv_ref, wphi_ref, wo_ref, win_ref, wsp_ref, bsp_ref, wout_ref, gout_ref,
            out_ref, dx_ref, dwqkv_ref, dwphi_ref, dwo_ref, dwin_ref, dwsp_ref, dbsp_ref,
            dwout_ref, spill_a, spill_b,
            xs, buf_a, buf_b, wcat, wcat_t, wop, wop_t, win_t, wout_t, bdp,
            dg_t, dg_n, dp_buf, small_acc, lq, lq_t, den_ref, rstd_ref,
            dwcat_acc, dwo_acc, dwin_acc, dwout_acc, dbsp_acc, sems):

    def lanes(ci):
        return pl.ds(pl.multiple_of(ci * C, C), C)

    def perm_mask():
        r = lax.broadcasted_iota(jnp.int32, (D, D), 0)
        c = lax.broadcasted_iota(jnp.int32, (D, D), 1)
        same_head = (r // DH) == (c // GR) * 8 + c % 8
        return same_head, same_head & ((r % DH) == (c % GR) // 8)

    def expand_mat():
        r = lax.broadcasted_iota(jnp.int32, (128, D), 0)
        c = lax.broadcasted_iota(jnp.int32, (128, D), 1)
        return jnp.where(r == (c % GR) // 8, 1.0, 0.0).astype(bf16)

    def group_mask():
        r = lax.broadcasted_iota(jnp.int32, (GA, 2 * GR), 0)
        c = lax.broadcasted_iota(jnp.int32, (GA, 2 * GR), 1)
        return ((r % 8) == (c % 8)) & (r < GR + 8)

    def eye320():
        r = lax.broadcasted_iota(jnp.int32, (2 * GR, 2 * GR), 0)
        c = lax.broadcasted_iota(jnp.int32, (2 * GR, 2 * GR), 1)
        return jnp.where(r == c, 1.0, 0.0).astype(bf16)

    same_head, pm = perm_mask()
    pmat = jnp.where(pm, 1.0, 0.0).astype(bf16)
    bdp_v = jnp.where(same_head, _nn(wphi_ref[...], expand_mat()), 0.0).astype(bf16)
    bdp[...] = bdp_v
    wc_q = _nn(wqkv_ref[:, 0:D], bdp_v)
    wcat[:, 0:D] = wc_q.astype(bf16)
    wcat_t[0:D, :] = wc_q.T.astype(bf16)
    wc_k = _nn(wqkv_ref[:, D:2 * D], bdp_v)
    wcat[:, D:2 * D] = wc_k.astype(bf16)
    wcat_t[D:2 * D, :] = wc_k.T.astype(bf16)
    wc_v = _nn(wqkv_ref[:, 2 * D:3 * D], pmat)
    wcat[:, 2 * D:3 * D] = wc_v.astype(bf16)
    wcat_t[2 * D:3 * D, :] = wc_v.T.astype(bf16)
    wo_tp = _nn(wo_ref[...].astype(f32).T.astype(bf16), pmat)
    wop_t[...] = wo_tp.astype(bf16)
    wop[...] = wo_tp.T.astype(bf16)
    win_t[...] = win_ref[...].astype(f32).T.astype(bf16)
    wout_t[...] = wout_ref[...].astype(f32).T.astype(bf16)
    for ci in range(NC):
        xs[:, ci * C:(ci + 1) * C] = x_ref[ci * C:(ci + 1) * C, :].astype(f32).T
    for g in range(NG):
        buf_a[A_V + g * GA + GR:A_V + (g + 1) * GA, :] = jnp.ones((GA - GR, S), bf16)

    def a_fwd(l):
        small_acc[...] = jnp.zeros(small_acc.shape, f32)

        def body1(ci, carry):
            ds = lanes(ci)
            xn, rstd = _ln_fwd(xs[:, ds])
            xnb = xn.astype(bf16)
            buf_a[A_XN:A_XN + D, ds] = xnb
            rstd_ref[2 * l:2 * l + 1, ds] = rstd
            pb = _nn(wcat_t[...], xnb).astype(bf16)
            buf_a[A_PQ:A_PQ + 2 * D, ds] = pb[0:2 * D]
            for g in range(NG):
                buf_a[A_V + g * GA:A_V + g * GA + GR, ds] = pb[2 * D + g * GR:2 * D + (g + 1) * GR]
                php, phn = _phi_pair(pb[D + g * GR:D + (g + 1) * GR].astype(f32))
                phik = _phi_cat(php, phn)
                small_acc[g] += _nt(buf_a[A_V + g * GA:A_V + (g + 1) * GA, ds], phik)
            return carry

        lax.fori_loop(0, NC, body1, 0)
        gm = group_mask()
        eye = eye320()
        for g in range(NG):
            lq_v = jnp.where(gm, small_acc[g], 0.0).astype(bf16)
            lq[l, g] = lq_v
            lq_t[l, g] = _nt(eye, lq_v).astype(bf16)

        def body2(ci, carry):
            ds = lanes(ci)
            for g in range(NG):
                php, phn = _phi_pair(buf_a[A_PQ + g * GR:A_PQ + (g + 1) * GR, ds].astype(f32))
                phiq = _phi_cat(php, phn)
                r = _nn(lq[l, g], phiq)
                den = r[GR:GR + 8] + 1e-6
                den_ref[l, 8 * g:8 * g + 8, ds] = den
                o = r[0:GR].reshape(DH, 8, C) / den[None]
                buf_a[A_O + g * GR:A_O + (g + 1) * GR, ds] = o.reshape(GR, C).astype(bf16)
            xs[:, ds] += _nn(wop_t[...], buf_a[A_O:A_O + D, ds])
            return carry

        lax.fori_loop(0, NC, body2, 0)

    def b_fwd(l):
        def body1(ci, carry):
            ds = lanes(ci)
            xn, rstd = _ln_fwd(xs[:, ds])
            xnb = xn.astype(bf16)
            buf_b[B_XN:B_XN + D, ds] = xnb
            rstd_ref[2 * l + 1:2 * l + 2, ds] = rstd
            hb = _nn(win_t[...], xnb).astype(bf16)
            buf_b[B_H:B_H + 2 * FH, ds] = hb
            z2n, rstd2 = _ln_fwd(_gelu(hb[FH:].astype(f32)))
            buf_b[B_Z2:B_Z2 + FH, ds] = z2n.astype(bf16)
            rstd_ref[4 + l:5 + l, ds] = rstd2
            return carry

        lax.fori_loop(0, NC, body1, 0)

        def body2(ci, carry):
            ds = lanes(ci)
            g = _nt(buf_b[B_Z2:B_Z2 + FH, :], wsp_ref[ds, :]) + bsp_ref[:, ds].astype(f32)
            gb = g.astype(bf16)
            buf_b[B_G:B_G + FH, ds] = gb
            z1 = _gelu(buf_b[B_H:B_H + FH, ds].astype(f32))
            u = (z1 * gb.astype(f32)).astype(bf16)
            xs[:, ds] += _nn(wout_t[...], u)
            return carry

        lax.fori_loop(0, NC, body2, 0)

    def b_bwd(l, first):
        def body1(ci, carry):
            ds = lanes(ci)
            doutb = xs[:, ds].astype(bf16)
            du = _nn(wout_ref[...], doutb)
            z1, dz1 = _gelu_and_grad(buf_b[B_H:B_H + FH, ds].astype(f32))
            g = buf_b[B_G:B_G + FH, ds].astype(f32)
            u = (z1 * g).astype(bf16)
            dwout_acc[...] += _nt(u, doutb)
            dg = du * z1
            dbsp_acc[:, ds] += jnp.sum(dg, axis=0, keepdims=True)
            dg_t[:, ds] = dg.astype(bf16)
            dg_n[ds, :] = dg.T.astype(bf16)
            buf_b[B_H:B_H + FH, ds] = (du * g * dz1).astype(bf16)
            return carry

        lax.fori_loop(0, NC, body1, 0)

        def body2(ci, carry):
            ds = lanes(ci)
            dz2 = _nn(dg_t[...], wsp_ref[:, ds])
            z2b = buf_b[B_Z2:B_Z2 + FH, ds]
            dpre = _ln_bwd(dz2, z2b.astype(f32), rstd_ref[4 + l:5 + l, ds])
            _, dge = _gelu_and_grad(buf_b[B_H + FH:B_H + 2 * FH, ds].astype(f32))
            buf_b[B_H + FH:B_H + 2 * FH, ds] = (dpre * dge).astype(bf16)
            dws = _nn(dg_n[...], z2b)
            if first:
                dwsp_ref[:, ds] = dws.astype(bf16)
            else:
                dwsp_ref[:, ds] = (dwsp_ref[:, ds].astype(f32) + dws).astype(bf16)
            dh = buf_b[B_H:B_H + 2 * FH, ds]
            xnb = buf_b[B_XN:B_XN + D, ds]
            dwin_acc[...] += _nt(xnb, dh)
            dxn = _nn(win_ref[...], dh)
            xs[:, ds] += _ln_bwd(dxn, xnb.astype(f32), rstd_ref[2 * l + 1:2 * l + 2, ds])
            return carry

        lax.fori_loop(0, NC, body2, 0)

    def a_bwd(l):
        small_acc[...] = jnp.zeros(small_acc.shape, f32)

        def body1(ci, carry):
            ds = lanes(ci)
            doutb = xs[:, ds].astype(bf16)
            do = _nn(wop[...], doutb)
            ob = buf_a[A_O:A_O + D, ds]
            dwo_acc[...] += _nt(ob, doutb)
            for g in range(NG):
                php, phn = _phi_pair(buf_a[A_PQ + g * GR:A_PQ + (g + 1) * GR, ds].astype(f32))
                phiq = _phi_cat(php, phn)
                den = den_ref[l, 8 * g:8 * g + 8, ds]
                dnum = do[g * GR:(g + 1) * GR].reshape(DH, 8, C) / den[None]
                o3 = ob[g * GR:(g + 1) * GR].astype(f32).reshape(DH, 8, C)
                dden = -jnp.sum(dnum * o3, axis=0)
                dnd = jnp.concatenate(
                    [dnum.reshape(GR, C), dden, jnp.zeros((8, C), f32)], axis=0).astype(bf16)
                dphi = _nn(lq_t[l, g], dnd)
                buf_a[A_PQ + g * GR:A_PQ + (g + 1) * GR, ds] = (
                    _softmax_pair_bwd(php, phn, dphi).astype(bf16))
                small_acc[g] += _nt(dnd, phiq)
            return carry

        lax.fori_loop(0, NC, body1, 0)
        gm = group_mask()
        eye = eye320()
        for g in range(NG):
            dl = jnp.where(gm, small_acc[g], 0.0).astype(bf16)
            lq[l, g] = dl
            lq_t[l, g] = _nt(eye, dl).astype(bf16)

        def body2(ci, carry):
            ds = lanes(ci)
            dp_buf[0:D, :] = buf_a[A_PQ:A_PQ + D, ds]
            for g in range(NG):
                php, phn = _phi_pair(buf_a[A_PK + g * GR:A_PK + (g + 1) * GR, ds].astype(f32))
                phik = _phi_cat(php, phn)
                dphi = _nn(lq_t[l, g], buf_a[A_V + g * GA:A_V + (g + 1) * GA, ds])
                dp_buf[D + g * GR:D + (g + 1) * GR, :] = (
                    _softmax_pair_bwd(php, phn, dphi).astype(bf16))
                dp_buf[2 * D + g * GR:2 * D + (g + 1) * GR, :] = (
                    _nn(lq[l, g, 0:GR, :], phik).astype(bf16))
            dp = dp_buf[...]
            xnb = buf_a[A_XN:A_XN + D, ds]
            dwcat_acc[...] += _nt(xnb, dp)
            dxn = _nn(wcat[...], dp)
            xs[:, ds] += _ln_bwd(dxn, xnb.astype(f32), rstd_ref[2 * l:2 * l + 1, ds])
            return carry

        lax.fori_loop(0, NC, body2, 0)

    cp_a_out = pltpu.make_async_copy(buf_a, spill_a, sems.at[0])
    cp_b_out = pltpu.make_async_copy(buf_b, spill_b, sems.at[1])
    cp_a_in = pltpu.make_async_copy(spill_a, buf_a, sems.at[2])
    cp_b_in = pltpu.make_async_copy(spill_b, buf_b, sems.at[3])

    a_fwd(0)
    cp_a_out.start()
    b_fwd(0)
    cp_b_out.start()
    cp_a_out.wait()
    a_fwd(1)
    cp_b_out.wait()
    b_fwd(1)

    for ci in range(NC):
        out_ref[ci * C:(ci + 1) * C, :] = xs[:, ci * C:(ci + 1) * C].T.astype(bf16)
        xs[:, ci * C:(ci + 1) * C] = gout_ref[ci * C:(ci + 1) * C, :].astype(f32).T
    dwcat_acc[...] = jnp.zeros(dwcat_acc.shape, f32)
    dwo_acc[...] = jnp.zeros(dwo_acc.shape, f32)
    dwin_acc[...] = jnp.zeros(dwin_acc.shape, f32)
    dwout_acc[...] = jnp.zeros(dwout_acc.shape, f32)
    dbsp_acc[...] = jnp.zeros(dbsp_acc.shape, f32)

    b_bwd(1, True)
    cp_b_in.start()
    a_bwd(1)
    cp_a_in.start()
    cp_b_in.wait()
    b_bwd(0, False)
    cp_a_in.wait()
    a_bwd(0)

    for ci in range(NC):
        dx_ref[ci * C:(ci + 1) * C, :] = xs[:, ci * C:(ci + 1) * C].T.astype(bf16)
    dwin_ref[...] = dwin_acc[...].astype(bf16)
    dwout_ref[...] = dwout_acc[...].astype(bf16)
    dbsp_ref[...] = dbsp_acc[...].astype(bf16)
    same_head, pm = perm_mask()
    pmat = jnp.where(pm, 1.0, 0.0).astype(bf16)
    dwo_ref[...] = _nn(pmat, dwo_acc[...].astype(bf16)).astype(bf16)
    dq = dwcat_acc[:, 0:D].astype(bf16)
    dk = dwcat_acc[:, D:2 * D].astype(bf16)
    dwqkv_ref[:, 0:D] = _nt(dq, bdp[...]).astype(bf16)
    dwqkv_ref[:, D:2 * D] = _nt(dk, bdp[...]).astype(bf16)
    dwqkv_ref[:, 2 * D:3 * D] = _nt(dwcat_acc[:, 2 * D:3 * D].astype(bf16), pmat).astype(bf16)
    wq_t = wqkv_ref[:, 0:D].astype(f32).T.astype(bf16)
    wk_t = wqkv_ref[:, D:2 * D].astype(f32).T.astype(bf16)
    dbd = jnp.where(same_head, _nn(wq_t, dq) + _nn(wk_t, dk), 0.0).astype(bf16)
    dwphi_ref[...] = _nt(dbd, expand_mat()).astype(bf16)


@jax.jit
def pallas_interleave_layers__linear_kernel_hedgehog__mixer_gmlp__prompt_kernel(
    A_x: jax.Array,
    A_wqkv: jax.Array,
    A_w_phi: jax.Array,
    A_wo: jax.Array,
    B_x: jax.Array,
    B_w_in: jax.Array,
    B_w_sp: jax.Array,
    B_b_sp: jax.Array,
    B_w_out: jax.Array,
    grad_out: jax.Array,
):
    x2 = A_x.reshape(S, D)
    g2 = grad_out.reshape(S, D)
    wphi2 = jnp.pad(A_w_phi.reshape(D, DH), ((0, 0), (0, 128 - DH)))
    bsp2 = B_b_sp.reshape(1, S)

    vm = pl.BlockSpec(memory_space=pltpu.VMEM)
    hbm = pl.BlockSpec(memory_space=pl.ANY)
    out_shape = (
        jax.ShapeDtypeStruct((S, D), bf16),
        jax.ShapeDtypeStruct((S, D), bf16),
        jax.ShapeDtypeStruct((D, 3 * D), bf16),
        jax.ShapeDtypeStruct((D, 128), bf16),
        jax.ShapeDtypeStruct((D, D), bf16),
        jax.ShapeDtypeStruct((D, 2 * FH), bf16),
        jax.ShapeDtypeStruct((S, S), bf16),
        jax.ShapeDtypeStruct((1, S), bf16),
        jax.ShapeDtypeStruct((FH, D), bf16),
        jax.ShapeDtypeStruct((A_ROWS, S), bf16),
        jax.ShapeDtypeStruct((B_ROWS, S), bf16),
    )
    scratch = [
        pltpu.VMEM((D, S), f32),
        pltpu.VMEM((A_ROWS, S), bf16),
        pltpu.VMEM((B_ROWS, S), bf16),
        pltpu.VMEM((D, 3 * D), bf16),
        pltpu.VMEM((3 * D, D), bf16),
        pltpu.VMEM((D, D), bf16),
        pltpu.VMEM((D, D), bf16),
        pltpu.VMEM((2 * FH, D), bf16),
        pltpu.VMEM((D, FH), bf16),
        pltpu.VMEM((D, D), bf16),
        pltpu.VMEM((FH, S), bf16),
        pltpu.VMEM((S, FH), bf16),
        pltpu.VMEM((3 * D, C), bf16),
        pltpu.VMEM((NG, GA, 2 * GR), f32),
        pltpu.VMEM((2, NG, GA, 2 * GR), bf16),
        pltpu.VMEM((2, NG, 2 * GR, GA), bf16),
        pltpu.VMEM((2, 32, S), f32),
        pltpu.VMEM((8, S), f32),
        pltpu.VMEM((D, 3 * D), f32),
        pltpu.VMEM((D, D), f32),
        pltpu.VMEM((D, 2 * FH), f32),
        pltpu.VMEM((FH, D), f32),
        pltpu.VMEM((1, S), f32),
        pltpu.SemaphoreType.DMA((4,)),
    ]
    res = pl.pallas_call(
        _kernel,
        out_shape=out_shape,
        in_specs=[vm] * 9,
        out_specs=tuple([vm] * 9 + [hbm, hbm]),
        scratch_shapes=scratch,
        compiler_params=pltpu.CompilerParams(vmem_limit_bytes=124 * 1024 * 1024),
    )(x2, A_wqkv, wphi2, A_wo, B_w_in, B_w_sp, bsp2, B_w_out, g2)
    out, dx, dwqkv, dwphi, dwo, dwin, dwsp, dbsp, dwout = res[:9]
    return (
        out.reshape(1, S, D),
        dx.reshape(1, S, D),
        dwqkv,
        dwphi[:, :DH].reshape(H, DH, DH),
        dwo,
        dwin,
        dwsp,
        dbsp.reshape(S),
        dwout,
    )
```

```python
import jax
import jax.numpy as jnp
from jax import lax
import jax.experimental.pallas as pl
import jax.experimental.pallas.tpu as pltpu

f32 = jnp.float32
bf16 = jnp.bfloat16

S = 2048
D = 640
H = 32
DH = 20
FH = 768
NG = 4
GR = 160
GA = 176
C = 512
NC = S // C
CS = dict(af1=512, af2=1024, bf1=1024, bf2=512, bb1=512, bb2=512, ab1=512, ab2=512)

A_XN, A_PQ, A_PK, A_O, A_V = 0, 640, 1280, 1920, 2560
A_ROWS = A_V + NG * GA
B_XN, B_H, B_Z2, B_G = 0, 640, 640 + 1536, 640 + 1536 + 768
B_ROWS = B_G + FH

_GC = 0.7978845608028654
_GA3 = 0.044715


def _nn(a, b):
    return jnp.dot(a, b, preferred_element_type=f32)


def _nt(a, b):
    return lax.dot_general(a, b, (((1,), (1,)), ((), ())), preferred_element_type=f32)


def _ln_fwd(x):
    mu = jnp.mean(x, axis=0, keepdims=True)
    xc = x - mu
    var = jnp.mean(xc * xc, axis=0, keepdims=True)
    rstd = lax.rsqrt(var + 1e-5)
    return xc * rstd, rstd


def _ln_bwd(dxn, xn, rstd):
    m1 = jnp.mean(dxn, axis=0, keepdims=True)
    m2 = jnp.mean(dxn * xn, axis=0, keepdims=True)
    return rstd * (dxn - m1 - xn * m2)


def _gelu(x):
    t = jnp.tanh(_GC * (x + _GA3 * (x * x * x)))
    return 0.5 * x * (1.0 + t)


def _gelu_and_grad(x):
    x2 = x * x
    t = jnp.tanh(_GC * (x + _GA3 * (x2 * x)))
    hp = 0.5 * (1.0 + t)
    y = x * hp
    dy = hp + 0.5 * x * (1.0 - t * t) * (_GC * (1.0 + 3.0 * _GA3 * x2))
    return y, dy


def _phi_pair(p):
    n = p.shape[-1]
    p3 = p.reshape(DH, 8, n)
    mx = jnp.max(p3, axis=0, keepdims=True)
    mn = jnp.min(p3, axis=0, keepdims=True)
    ep = jnp.exp(p3 - mx)
    en = jnp.exp(mn - p3)
    sp = jnp.sum(ep, axis=0, keepdims=True)
    sn = jnp.sum(en, axis=0, keepdims=True)
    return ep * (1.0 / sp), en * (1.0 / sn)


def _phi_cat(php, phn):
    n = php.shape[-1]
    return jnp.concatenate(
        [php.reshape(GR, n).astype(bf16), phn.reshape(GR, n).astype(bf16)], axis=0)


def _softmax_pair_bwd(php, phn, dphi):
    n = dphi.shape[-1]
    dp_ = dphi[:GR].reshape(DH, 8, n)
    dn_ = dphi[GR:].reshape(DH, 8, n)
    sp = jnp.sum(php * dp_, axis=0, keepdims=True)
    sn = jnp.sum(phn * dn_, axis=0, keepdims=True)
    return (php * (dp_ - sp) - phn * (dn_ - sn)).reshape(GR, n)


def _kernel(x_hbm, wqkv_hbm, wphi_hbm, wo_hbm, win_hbm, wsp_hbm, bsp_hbm, wout_hbm, gout_hbm,
            out_hbm, dx_hbm, dwqkv_hbm, dwphi_hbm, dwo_hbm, dwin_hbm, dwsp_hbm, dbsp_hbm,
            dwout_hbm, spill_a, spill_b,
            x_ref, wqkv_ref, wphi_ref, wo_ref, win_ref, wsp_ref, bsp_ref, wout_ref, gout_ref,
            out_ref, dx_ref, dwqkv_ref, dwphi_ref, dwo_ref, dwin_ref, dwsp_ref, dbsp_ref,
            dwout_ref, isems, osems, csems,
            xs, buf_a, buf_b, wcat, wcat_t, wqkv_t, wop, wop_t, win_t, wout_t, bdp,
            dg_t, dg_n, dp_buf, small_acc, lq, lq_t, den_ref, rstd_ref,
            dwcat_acc, dwo_acc, dwin_acc, dwout_acc, dbsp_acc, sems):

    def lanes(ci, cs=C):
        return pl.ds(pl.multiple_of(ci * cs, cs), cs)

    def run(name, body):
        cs = CS[name]
        with jax.named_scope(name):
            lax.fori_loop(0, S // cs, lambda ci, c: body(ci, c, cs), 0)

    in_pairs = [(wphi_hbm, wphi_ref), (wqkv_hbm, wqkv_ref), (x_hbm, x_ref), (wo_hbm, wo_ref),
                (win_hbm, win_ref), (wsp_hbm, wsp_ref), (bsp_hbm, bsp_ref), (wout_hbm, wout_ref),
                (gout_hbm, gout_ref)]
    cin = [pltpu.make_async_copy(a, b, isems.at[i]) for i, (a, b) in enumerate(in_pairs)]
    out_pairs = [(dwqkv_ref, dwqkv_hbm), (dwphi_ref, dwphi_hbm), (dwo_ref, dwo_hbm),
                 (dwin_ref, dwin_hbm), (dwsp_ref, dwsp_hbm), (dbsp_ref, dbsp_hbm),
                 (dwout_ref, dwout_hbm)]
    cout = [pltpu.make_async_copy(a, b, osems.at[i]) for i, (a, b) in enumerate(out_pairs)]

    def chunk_copy(which, ci):
        cs = CS[("bf2", "ab2")[which]]
        src, dst = ((out_ref, out_hbm), (dx_ref, dx_hbm))[which]
        return pltpu.make_async_copy(src.at[lanes(ci, cs), :], dst.at[lanes(ci, cs), :],
                                     csems.at[which * 8 + ci])

    for i in range(4):
        cin[i].start()

    def blk_consts():
        r = lax.broadcasted_iota(jnp.int32, (GR, GR), 0)
        j = lax.broadcasted_iota(jnp.int32, (GR, GR), 1)
        same_rj = (r // DH) == (j % 8)
        p_rj = jnp.where(same_rj & ((r % DH) == (j // 8)), 1.0, 0.0).astype(bf16)
        same_jr = (j // DH) == (r % 8)
        p_jr = jnp.where(same_jr & ((j % DH) == (r // 8)), 1.0, 0.0).astype(bf16)
        eye = jnp.where(r == j, 1.0, 0.0).astype(bf16)
        return same_rj, p_rj, p_jr, eye

    def expand_mat():
        r = lax.broadcasted_iota(jnp.int32, (128, GR), 0)
        c = lax.broadcasted_iota(jnp.int32, (128, GR), 1)
        return jnp.where(r == c // 8, 1.0, 0.0).astype(bf16)

    def group_mask():
        r = lax.broadcasted_iota(jnp.int32, (GA, 2 * GR), 0)
        c = lax.broadcasted_iota(jnp.int32, (GA, 2 * GR), 1)
        return ((r % 8) == (c % 8)) & (r < GR + 8)

    def eye320():
        r = lax.broadcasted_iota(jnp.int32, (2 * GR, 2 * GR), 0)
        c = lax.broadcasted_iota(jnp.int32, (2 * GR, 2 * GR), 1)
        return jnp.where(r == c, 1.0, 0.0).astype(bf16)

    with jax.named_scope("prep"):
        cin[0].wait()
        cin[1].wait()
        same_rj, p_rj, p_jr, eye = blk_consts()
        e_perm = expand_mat()
        wqkv_t[...] = wqkv_ref[...].astype(f32).T.astype(bf16)
        for g in range(NG):
            rows = slice(g * GR, (g + 1) * GR)
            bd = jnp.where(same_rj, _nn(wphi_ref[rows, :], e_perm), 0.0).astype(bf16)
            bdp[rows, :] = bd
            bdt = _nt(eye, bd).astype(bf16)
            wcat_t[g * GR:(g + 1) * GR, :] = _nn(bdt, wqkv_t[g * GR:(g + 1) * GR, :]).astype(bf16)
            wcat_t[D + g * GR:D + (g + 1) * GR, :] = (
                _nn(bdt, wqkv_t[D + g * GR:D + (g + 1) * GR, :]).astype(bf16))
            wcat_t[2 * D + g * GR:2 * D + (g + 1) * GR, :] = (
                _nn(p_jr, wqkv_t[2 * D + g * GR:2 * D + (g + 1) * GR, :]).astype(bf16))
        wcat[...] = wcat_t[...].astype(f32).T.astype(bf16)
        cin[2].wait()
        cin[3].wait()
        for i in range(4, 9):
            cin[i].start()
        for g in range(NG):
            wop[g * GR:(g + 1) * GR, :] = _nn(p_jr, wo_ref[g * GR:(g + 1) * GR, :]).astype(bf16)
        wop_t[...] = wop[...].astype(f32).T.astype(bf16)
        for ci in range(NC):
            xs[:, ci * C:(ci + 1) * C] = x_ref[ci * C:(ci + 1) * C, :].astype(f32).T
        for g in range(NG):
            buf_a[A_V + g * GA + GR:A_V + (g + 1) * GA, :] = jnp.ones((GA - GR, S), bf16)

    def a_fwd(l):
        small_acc[...] = jnp.zeros(small_acc.shape, f32)

        def body1(ci, carry, C):
            ds = lanes(ci, C)
            xn, rstd = _ln_fwd(xs[:, ds])
            xnb = xn.astype(bf16)
            buf_a[A_XN:A_XN + D, ds] = xnb
            rstd_ref[2 * l:2 * l + 1, ds] = rstd
            pb = _nn(wcat_t[...], xnb).astype(bf16)
            buf_a[A_PQ:A_PQ + 2 * D, ds] = pb[0:2 * D]
            for g in range(NG):
                buf_a[A_V + g * GA:A_V + g * GA + GR, ds] = pb[2 * D + g * GR:2 * D + (g + 1) * GR]
                php, phn = _phi_pair(pb[D + g * GR:D + (g + 1) * GR].astype(f32))
                phik = _phi_cat(php, phn)
                small_acc[g] += _nt(buf_a[A_V + g * GA:A_V + (g + 1) * GA, ds], phik)
            return carry

        run("af1", body1)
        gm = group_mask()
        eye = eye320()
        for g in range(NG):
            lq_v = jnp.where(gm, small_acc[g], 0.0).astype(bf16)
            lq[l, g] = lq_v
            lq_t[l, g] = _nt(eye, lq_v).astype(bf16)

        def body2(ci, carry, C):
            ds = lanes(ci, C)
            for g in range(NG):
                php, phn = _phi_pair(buf_a[A_PQ + g * GR:A_PQ + (g + 1) * GR, ds].astype(f32))
                phiq = _phi_cat(php, phn)
                r = _nn(lq[l, g], phiq)
                den = r[GR:GR + 8] + 1e-6
                den_ref[l, 8 * g:8 * g + 8, ds] = den
                o = r[0:GR].reshape(DH, 8, C) / den[None]
                buf_a[A_O + g * GR:A_O + (g + 1) * GR, ds] = o.reshape(GR, C).astype(bf16)
            xs[:, ds] += _nn(wop_t[...], buf_a[A_O:A_O + D, ds])
            return carry

        run("af2", body2)

    def b_fwd(l, last):
        def body1(ci, carry, C):
            ds = lanes(ci, C)
            xn, rstd = _ln_fwd(xs[:, ds])
            xnb = xn.astype(bf16)
            buf_b[B_XN:B_XN + D, ds] = xnb
            rstd_ref[2 * l + 1:2 * l + 2, ds] = rstd
            hb = _nn(win_t[...], xnb).astype(bf16)
            buf_b[B_H:B_H + 2 * FH, ds] = hb
            z2n, rstd2 = _ln_fwd(_gelu(hb[FH:].astype(f32)))
            buf_b[B_Z2:B_Z2 + FH, ds] = z2n.astype(bf16)
            rstd_ref[4 + l:5 + l, ds] = rstd2
            return carry

        run("bf1", body1)

        def body2(ci, carry, C):
            ds = lanes(ci, C)
            g = _nt(buf_b[B_Z2:B_Z2 + FH, :], wsp_ref[ds, :]) + bsp_ref[:, ds].astype(f32)
            gb = g.astype(bf16)
            buf_b[B_G:B_G + FH, ds] = gb
            z1 = _gelu(buf_b[B_H:B_H + FH, ds].astype(f32))
            u = (z1 * gb.astype(f32)).astype(bf16)
            y = xs[:, ds] + _nn(wout_t[...], u)
            if last:
                out_ref[ds, :] = y.T.astype(bf16)
                chunk_copy(0, ci).start()
                xs[:, ds] = gout_ref[ds, :].astype(f32).T
            else:
                xs[:, ds] = y
            return carry

        run("bf2", body2)

    def b_bwd(l, first):
        def body1(ci, carry, C):
            ds = lanes(ci, C)
            doutb = xs[:, ds].astype(bf16)
            du = _nn(wout_ref[...], doutb)
            z1, dz1 = _gelu_and_grad(buf_b[B_H:B_H + FH, ds].astype(f32))
            g = buf_b[B_G:B_G + FH, ds].astype(f32)
            u = (z1 * g).astype(bf16)
            dg = du * z1
            dbsp_acc[:, ds] += jnp.sum(dg, axis=0, keepdims=True)
            dg_t[:, ds] = dg.astype(bf16)
            dg_n[ds, :] = dg.T.astype(bf16)
            buf_b[B_H:B_H + FH, ds] = (du * g * dz1).astype(bf16)
            dwout_acc[...] += _nt(u, doutb)
            return carry

        run("bb1", body1)

        def body2(ci, carry, C):
            ds = lanes(ci, C)
            dz2 = _nn(dg_t[...], wsp_ref[:, ds])
            z2b = buf_b[B_Z2:B_Z2 + FH, ds]
            dpre = _ln_bwd(dz2, z2b.astype(f32), rstd_ref[4 + l:5 + l, ds])
            _, dge = _gelu_and_grad(buf_b[B_H + FH:B_H + 2 * FH, ds].astype(f32))
            buf_b[B_H + FH:B_H + 2 * FH, ds] = (dpre * dge).astype(bf16)
            dh = buf_b[B_H:B_H + 2 * FH, ds]
            xnb = buf_b[B_XN:B_XN + D, ds]
            dxn = _nn(win_ref[...], dh)
            xs[:, ds] += _ln_bwd(dxn, xnb.astype(f32), rstd_ref[2 * l + 1:2 * l + 2, ds])
            dwin_acc[...] += _nt(xnb, dh)
            dws = _nn(dg_n[...], z2b)
            if first:
                dwsp_ref[:, ds] = dws.astype(bf16)
            else:
                dwsp_ref[:, ds] = (dwsp_ref[:, ds].astype(f32) + dws).astype(bf16)
            return carry

        run("bb2", body2)

    def a_bwd(l, last):
        small_acc[...] = jnp.zeros(small_acc.shape, f32)

        def body1(ci, carry, C):
            ds = lanes(ci, C)
            doutb = xs[:, ds].astype(bf16)
            do = _nn(wop[...], doutb)
            ob = buf_a[A_O:A_O + D, ds]
            for g in range(NG):
                php, phn = _phi_pair(buf_a[A_PQ + g * GR:A_PQ + (g + 1) * GR, ds].astype(f32))
                phiq = _phi_cat(php, phn)
                den = den_ref[l, 8 * g:8 * g + 8, ds]
                dnum = do[g * GR:(g + 1) * GR].reshape(DH, 8, C) / den[None]
                o3 = ob[g * GR:(g + 1) * GR].astype(f32).reshape(DH, 8, C)
                dden = -jnp.sum(dnum * o3, axis=0)
                dnd = jnp.concatenate(
                    [dnum.reshape(GR, C), dden, jnp.zeros((8, C), f32)], axis=0).astype(bf16)
                dphi = _nn(lq_t[l, g], dnd)
                buf_a[A_PQ + g * GR:A_PQ + (g + 1) * GR, ds] = (
                    _softmax_pair_bwd(php, phn, dphi).astype(bf16))
                small_acc[g] += _nt(dnd, phiq)
            dwo_acc[...] += _nt(ob, doutb)
            return carry

        run("ab1", body1)
        gm = group_mask()
        eye = eye320()
        for g in range(NG):
            dl = jnp.where(gm, small_acc[g], 0.0).astype(bf16)
            lq[l, g] = dl
            lq_t[l, g] = _nt(eye, dl).astype(bf16)

        def body2(ci, carry, C):
            ds = lanes(ci, C)
            dp_buf[0:D, :] = buf_a[A_PQ:A_PQ + D, ds]
            for g in range(NG):
                php, phn = _phi_pair(buf_a[A_PK + g * GR:A_PK + (g + 1) * GR, ds].astype(f32))
                phik = _phi_cat(php, phn)
                dphi = _nn(lq_t[l, g], buf_a[A_V + g * GA:A_V + (g + 1) * GA, ds])
                dp_buf[D + g * GR:D + (g + 1) * GR, :] = (
                    _softmax_pair_bwd(php, phn, dphi).astype(bf16))
                dp_buf[2 * D + g * GR:2 * D + (g + 1) * GR, :] = (
                    _nn(lq[l, g, 0:GR, :], phik).astype(bf16))
            dp = dp_buf[...]
            xnb = buf_a[A_XN:A_XN + D, ds]
            dxn = _nn(wcat[...], dp)
            y = xs[:, ds] + _ln_bwd(dxn, xnb.astype(f32), rstd_ref[2 * l:2 * l + 1, ds])
            if last:
                dx_ref[ds, :] = y.T.astype(bf16)
            else:
                xs[:, ds] = y
            dwcat_acc[...] += _nt(dp, xnb)
            if last:
                chunk_copy(1, ci).start()
            return carry

        run("ab2", body2)

    cp_a_out = pltpu.make_async_copy(buf_a, spill_a, sems.at[0])
    cp_b_out = pltpu.make_async_copy(buf_b, spill_b, sems.at[1])
    cp_a_in = pltpu.make_async_copy(spill_a, buf_a, sems.at[2])
    cp_b_in = pltpu.make_async_copy(spill_b, buf_b, sems.at[3])

    a_fwd(0)
    cp_a_out.start()
    for i in range(4, 9):
        cin[i].wait()
    win_t[...] = win_ref[...].astype(f32).T.astype(bf16)
    wout_t[...] = wout_ref[...].astype(f32).T.astype(bf16)
    b_fwd(0, False)
    cp_b_out.start()
    cp_a_out.wait()
    a_fwd(1)
    cp_b_out.wait()
    b_fwd(1, True)

    with jax.named_scope("mid"):
        dwcat_acc[...] = jnp.zeros(dwcat_acc.shape, f32)
        dwo_acc[...] = jnp.zeros(dwo_acc.shape, f32)
        dwin_acc[...] = jnp.zeros(dwin_acc.shape, f32)
        dwout_acc[...] = jnp.zeros(dwout_acc.shape, f32)
        dbsp_acc[...] = jnp.zeros(dbsp_acc.shape, f32)

    b_bwd(1, True)
    cp_b_in.start()
    a_bwd(1, False)
    cp_a_in.start()
    cp_b_in.wait()
    b_bwd(0, False)
    dwin_ref[...] = dwin_acc[...].astype(bf16)
    dwout_ref[...] = dwout_acc[...].astype(bf16)
    dbsp_ref[...] = dbsp_acc[...].astype(bf16)
    for i in range(3, 7):
        cout[i].start()
    cp_a_in.wait()
    a_bwd(0, True)

    with jax.named_scope("epi"):
        same_rj, p_rj, _, _ = blk_consts()
        e_perm = expand_mat()
        for g in range(NG):
            rows = slice(g * GR, (g + 1) * GR)
            dwo_ref[rows, :] = _nn(p_rj, dwo_acc[rows, :].astype(bf16)).astype(bf16)
        cout[2].start()
        for g in range(NG):
            rows = slice(g * GR, (g + 1) * GR)
            dq = dwcat_acc[g * GR:(g + 1) * GR, :].astype(bf16)
            dk = dwcat_acc[D + g * GR:D + (g + 1) * GR, :].astype(bf16)
            dv = dwcat_acc[2 * D + g * GR:2 * D + (g + 1) * GR, :].astype(bf16)
            bd = bdp[rows, :]
            dbd = (_nt(wqkv_t[g * GR:(g + 1) * GR, :], dq)
                   + _nt(wqkv_t[D + g * GR:D + (g + 1) * GR, :], dk))
            dbd = jnp.where(same_rj, dbd, 0.0).astype(bf16)
            dwphi_ref[rows, :] = _nt(dbd, e_perm).astype(bf16)
            dwcat_acc[g * GR:(g + 1) * GR, :] = _nn(bd, dq)
            dwcat_acc[D + g * GR:D + (g + 1) * GR, :] = _nn(bd, dk)
            dwcat_acc[2 * D + g * GR:2 * D + (g + 1) * GR, :] = _nn(p_rj, dv)
        dwqkv_ref[...] = dwcat_acc[...].T.astype(bf16)
        cout[0].start()
        cout[1].start()
        for i in range(7):
            cout[i].wait()
        for w in range(2):
            for ci in range(S // CS[("bf2", "ab2")[w]]):
                chunk_copy(w, ci).wait()


@jax.jit
def pallas_interleave_layers__linear_kernel_hedgehog__mixer_gmlp__prompt_kernel(
    A_x: jax.Array,
    A_wqkv: jax.Array,
    A_w_phi: jax.Array,
    A_wo: jax.Array,
    B_x: jax.Array,
    B_w_in: jax.Array,
    B_w_sp: jax.Array,
    B_b_sp: jax.Array,
    B_w_out: jax.Array,
    grad_out: jax.Array,
):
    x2 = A_x.reshape(S, D)
    g2 = grad_out.reshape(S, D)
    wphi2 = jnp.pad(A_w_phi.reshape(D, DH), ((0, 0), (0, 128 - DH)))
    bsp2 = B_b_sp.reshape(1, S)

    hbm = pl.BlockSpec(memory_space=pl.ANY)
    out_shape = (
        jax.ShapeDtypeStruct((S, D), bf16),
        jax.ShapeDtypeStruct((S, D), bf16),
        jax.ShapeDtypeStruct((D, 3 * D), bf16),
        jax.ShapeDtypeStruct((D, 128), bf16),
        jax.ShapeDtypeStruct((D, D), bf16),
        jax.ShapeDtypeStruct((D, 2 * FH), bf16),
        jax.ShapeDtypeStruct((S, S), bf16),
        jax.ShapeDtypeStruct((1, S), bf16),
        jax.ShapeDtypeStruct((FH, D), bf16),
        jax.ShapeDtypeStruct((A_ROWS, S), bf16),
        jax.ShapeDtypeStruct((B_ROWS, S), bf16),
    )
    ins = (x2, A_wqkv, wphi2, A_wo, B_w_in, B_w_sp, bsp2, B_w_out, g2)
    scratch = [pltpu.VMEM(a.shape, bf16) for a in ins]
    scratch += [pltpu.VMEM(o.shape, bf16) for o in out_shape[:9]]
    scratch += [
        pltpu.SemaphoreType.DMA((9,)),
        pltpu.SemaphoreType.DMA((7,)),
        pltpu.SemaphoreType.DMA((16,)),
        pltpu.VMEM((D, S), f32),
        pltpu.VMEM((A_ROWS, S), bf16),
        pltpu.VMEM((B_ROWS, S), bf16),
        pltpu.VMEM((D, 3 * D), bf16),
        pltpu.VMEM((3 * D, D), bf16),
        pltpu.VMEM((3 * D, D), bf16),
        pltpu.VMEM((D, D), bf16),
        pltpu.VMEM((D, D), bf16),
        pltpu.VMEM((2 * FH, D), bf16),
        pltpu.VMEM((D, FH), bf16),
        pltpu.VMEM((D, GR), bf16),
        pltpu.VMEM((FH, S), bf16),
        pltpu.VMEM((S, FH), bf16),
        pltpu.VMEM((3 * D, CS['ab2']), bf16),
        pltpu.VMEM((NG, GA, 2 * GR), f32),
        pltpu.VMEM((2, NG, GA, 2 * GR), bf16),
        pltpu.VMEM((2, NG, 2 * GR, GA), bf16),
        pltpu.VMEM((2, 32, S), f32),
        pltpu.VMEM((8, S), f32),
        pltpu.VMEM((3 * D, D), f32),
        pltpu.VMEM((D, D), f32),
        pltpu.VMEM((D, 2 * FH), f32),
        pltpu.VMEM((FH, D), f32),
        pltpu.VMEM((1, S), f32),
        pltpu.SemaphoreType.DMA((4,)),
    ]
    res = pl.pallas_call(
        _kernel,
        out_shape=out_shape,
        in_specs=[hbm] * 9,
        out_specs=tuple([hbm] * 11),
        scratch_shapes=scratch,
        compiler_params=pltpu.CompilerParams(vmem_limit_bytes=124 * 1024 * 1024),
    )(*ins)
    out, dx, dwqkv, dwphi, dwo, dwin, dwsp, dbsp, dwout = res[:9]
    return (
        out.reshape(1, S, D),
        dx.reshape(1, S, D),
        dwqkv,
        dwphi[:, :DH].reshape(H, DH, DH),
        dwo,
        dwin,
        dwsp,
        dbsp.reshape(S),
        dwout,
    )
```
